```python
import jax
import jax.numpy as jnp

def _softmax(x, axis=-1):
    return jax.nn.softmax(x, axis=axis)
def _gelu(x):
    return jax.nn.gelu(x, approximate=True)
def _silu(x):
    return jax.nn.silu(x)
def _sigmoid(x):
    return jax.nn.sigmoid(x)
def _layernorm(x, axis=-1, eps=1e-5):
    m = jnp.mean(x, axis=axis, keepdims=True)
    v = jnp.var(x, axis=axis, keepdims=True)
    return (x - m) / jnp.sqrt(v + eps)
def _scatter_add(tgt, idx, src, axis=0):
    return tgt.at[idx].add(src)
def _segment_sum(src, seg, n):
    return jax.ops.segment_sum(src, seg, n)
class _Rng:
    def __init__(self, key):
        self._k = key
    def _next(self):
        self._k, sub = jax.random.split(self._k)
        return sub
    def normal(self, shape):
        return jax.random.normal(self._next(), shape, dtype=jnp.bfloat16)
    def randint(self, lo, hi, shape):
        return jax.random.randint(self._next(), shape, lo, hi, dtype=jnp.int32)
    def uniform(self, shape, lo=0.0, hi=1.0):
        return jax.random.uniform(self._next(), shape, jnp.bfloat16, lo, hi)
    def permutation(self, n):
        return jax.random.permutation(self._next(), n)


kernel_name = 'recurrent_scan__compressed_kv_cla__dense_activation_gelu__decode'

def setup_inputs():
    _rng = _Rng(jax.random.key(int.from_bytes(__import__("os").urandom(4), "little")))
    _w = (lambda a: (lambda t: t.astype(jnp.bfloat16) if jnp.issubdtype(t.dtype, jnp.floating) else t)(jnp.asarray(a)))
    def _A_setup():
        B, H, Sq, Sk, D, M = 2, 32, 1, 16384, 128, 512
        Dc = 4 * D
        return {
            "x": _w((lambda *s: _rng.normal(s) * 0.05)(B, Sq, M)),
            "c_kv": _w((lambda *s: _rng.normal(s) * 0.05)(B, Sk, Dc)),
            "w_q": _w((lambda *s: _rng.normal(s) * 0.05)(M, H, D) * (M ** -0.5)),
            "w_uk": _w((lambda *s: _rng.normal(s) * 0.05)(Dc, H, D) * (Dc ** -0.5)),
            "w_uv": _w((lambda *s: _rng.normal(s) * 0.05)(Dc, H, D) * (Dc ** -0.5)),
            "w_o": _w((lambda *s: _rng.normal(s) * 0.05)(H, D, M) * ((H * D) ** -0.5)),
        }
    _A_in = _A_setup()

    def _B_setup():
        B, S, D, F = 2, 1, 512, 1792
        return {
            "x": _w((lambda *s: _rng.normal(s) * 0.05)(B, S, D)),
            "w1": _w((lambda *s: _rng.normal(s) * 0.05)(D, F) * (D ** -0.5)),
            "b1": _w((lambda *s: _rng.normal(s) * 0.05)(F) * 0.01),
            "w2": _w((lambda *s: _rng.normal(s) * 0.05)(F, D) * (F ** -0.5)),
            "b2": _w((lambda *s: _rng.normal(s) * 0.05)(D) * 0.01),
        }
    _B_in = _B_setup()

    return {
        "A_x": _A_in["x"],
        "A_c_kv": _A_in["c_kv"],
        "A_w_q": _A_in["w_q"],
        "A_w_uk": _A_in["w_uk"],
        "A_w_uv": _A_in["w_uv"],
        "A_w_o": _A_in["w_o"],
        "B_x": _B_in["x"],
        "B_w1": _B_in["w1"],
        "B_b1": _B_in["b1"],
        "B_w2": _B_in["w2"],
        "B_b2": _B_in["b2"],
    }

def reference(A_x, A_c_kv, A_w_q, A_w_uk, A_w_uv, A_w_o, B_x, B_w1, B_b1, B_w2, B_b2):
    def _A_ref(x, c_kv, w_q, w_uk, w_uv, w_o):
        B, Sq, M = x.shape[0], x.shape[1], x.shape[2]
        Sk = c_kv.shape[1]
        H, D = w_q.shape[1], w_q.shape[2]
        q = jnp.einsum("bqm,mhd->bhqd", x, w_q)
        k = jnp.einsum("bkc,chd->bhkd", c_kv, w_uk)
        v = jnp.einsum("bkc,chd->bhkd", c_kv, w_uv)
        scores = jnp.einsum("bhqd,bhkd->bhqk", q, k) * (D ** -0.5)
        off = Sk - Sq
        qi = jnp.arange(Sq)[:, None]
        kj = jnp.arange(Sk)[None, :]
        cmask = kj <= (qi + off)
        scores = jnp.where(cmask[None, None], scores, -1e9)
        p = _softmax(scores, axis=-1)
        ctx = jnp.einsum("bhqk,bhkd->bhqd", p, v)
        return jnp.einsum("bhqd,hdm->bqm", ctx, w_o)

    def _B_ref(x, w1, b1, w2, b2):
        h = jnp.einsum("bsd,df->bsf", x, w1) + b1
        h = _gelu(h)
        return jnp.einsum("bsf,fd->bsd", h, w2) + b2

    x = A_x
    xn = _layernorm(x, axis=-1)
    s = _A_ref(xn, A_c_kv, A_w_q, A_w_uk, A_w_uv, A_w_o)
    g = _silu(_B_ref(xn, B_w1, B_b1, B_w2, B_b2))
    return x + s * g
```

```python
import functools
import jax
import jax.numpy as jnp
import numpy as np
from jax import lax
import jax.experimental.pallas as pl
import jax.experimental.pallas.tpu as pltpu

F32 = jnp.float32
BF16 = jnp.bfloat16

B, H, SK, D, M, DC, F = 2, 32, 16384, 128, 512, 512, 1792


def make_kernel(BK=2048, AHEAD=3, UNROLL_Q=8):
    NKB = SK // BK

    def kernel(x_hbm, ckv_hbm, wq_hbm, wuk_hbm, wuv_hbm, wo_hbm, w1_hbm, b1_hbm, w2_hbm, b2_hbm,
               o_ref,
               x_buf, b1_buf, b2_buf, c_buf, wq_buf, wuk_buf, wuv_buf, wo_buf, w1_buf, w2_buf,
               xn_v, xs, t8, qa_ref, acc_ref, m_ref, l_ref, a_buf, sems, sem_small):
        copies = []
        def add(src, dst):
            copies.append(pltpu.make_async_copy(src, dst, sems.at[len(copies)]))
            return len(copies) - 1
        i_wq = [add(wq_hbm.at[pl.ds(j * 128, 128)], wq_buf.at[pl.ds(j * 128, 128)]) for j in range(4)]
        i_wuk = [add(wuk_hbm.at[pl.ds(j * 128, 128)], wuk_buf.at[pl.ds(j * 128, 128)]) for j in range(4)]
        i_c = [[add(ckv_hbm.at[b, pl.ds(j * BK, BK)], c_buf.at[b, pl.ds(j * BK, BK)]) for j in range(NKB)] for b in range(B)]
        i_wuv = [add(wuv_hbm.at[pl.ds(j * 128, 128)], wuv_buf.at[pl.ds(j * 128, 128)]) for j in range(4)]
        i_wo = [add(wo_hbm.at[pl.ds(j * 8, 8)], wo_buf.at[pl.ds(j * 8, 8)]) for j in range(4)]
        i_w1 = [add(w1_hbm.at[pl.ds(j * 256, 256)], w1_buf.at[pl.ds(j * 256, 256)]) for j in range(2)]
        i_w2 = [add(w2_hbm.at[pl.ds(j * 256, 256)], w2_buf.at[pl.ds(j * 256, 256)]) for j in range(7)]
        ncop = len(copies)
        small = [pltpu.make_async_copy(x_hbm, x_buf, sem_small.at[0]),
                 pltpu.make_async_copy(b1_hbm, b1_buf, sem_small.at[1]),
                 pltpu.make_async_copy(b2_hbm, b2_buf, sem_small.at[2])]
        started = [0]
        def start_upto(n):
            n = min(n, ncop)
            while started[0] < n:
                copies[started[0]].start()
                started[0] += 1
        def wait(i):
            copies[i].wait()
            start_upto(i + 1 + AHEAD)

        copies[0].start(); started[0] = 1
        small[0].start()
        start_upto(AHEAD)
        small[1].start(); small[2].start()

        small[0].wait()
        x = x_buf[...].astype(F32)
        mu = jnp.mean(x, axis=-1, keepdims=True)
        xc = x - mu
        var = jnp.mean(xc * xc, axis=-1, keepdims=True)
        xn = xc * lax.rsqrt(var + 1e-5)
        xn_b = xn.astype(BF16)
        xn_v[...] = xn_b.astype(F32)
        cp = pltpu.make_async_copy(xn_v, xs, sem_small.at[3])
        cp.start(); cp.wait()

        carry = (jnp.zeros((H, D), F32), jnp.zeros((H, D), F32))
        for j in range(4):
            wait(i_wq[j])
            def body(i, carry, j=j):
                a0, a1 = carry
                for u in range(UNROLL_Q):
                    m = j * 128 + i * UNROLL_Q + u
                    w = wq_buf[m].astype(F32)
                    a0 = a0 + xs[0, m] * w
                    a1 = a1 + xs[1, m] * w
                return a0, a1
            carry = lax.fori_loop(0, 128 // UNROLL_Q, body, carry)
        q = jnp.concatenate([carry[0], carry[1], jnp.zeros((64, D), F32)], axis=0).astype(BF16)

        lane3 = lax.broadcasted_iota(jnp.int32, (16, 8, 128), 2)
        g3 = (lane3 % 32) // 8
        for j in range(4):
            wait(i_wuk[j])
            for s in range(8):
                c0 = j * 128 + s * 16
                u = wuk_buf[pl.ds(c0, 16)].reshape(16 * 32, D)
                r = lax.dot_general(u, q, (((1,), (1,)), ((), ())), preferred_element_type=F32)
                r4 = r.reshape(16, 4, 8, 128)
                v = jnp.where(g3 == 0, r4[:, 0], jnp.where(g3 == 1, r4[:, 1], jnp.where(g3 == 2, r4[:, 2], r4[:, 3])))
                t8[pl.ds(c0 * 8, 128), :] = v.reshape(128, 128)
        lane2 = lax.broadcasted_iota(jnp.int32, (128, 128), 1) % 8
        scale = (D ** -0.5) * 1.4426950408889634
        for j in range(4):
            t = t8[pl.ds(j * 1024, 128, stride=8), :]
            for s in range(1, 8):
                t = jnp.where(lane2 == s, t8[pl.ds(j * 1024 + s, 128, stride=8), :], t)
            tt = t.T
            qa_ref[:, j * 128:(j + 1) * 128] = (tt[:64] * scale).astype(BF16)

        for b in range(B):
            rows = pl.ds(b * H, H)
            m_ref[rows, :] = jnp.full((H, 128), -1e30, F32)
            l_ref[rows, :] = jnp.zeros((H, 128), F32)
            acc_ref[rows, :] = jnp.zeros((H, DC), F32)
            for j in range(NKB):
                wait(i_c[b][j])
                qa = qa_ref[rows, :]
                c = c_buf[b, pl.ds(j * BK, BK), :]
                sc = lax.dot_general(qa, c, (((1,), (1,)), ((), ())), preferred_element_type=F32)
                m_prev = m_ref[rows, :]
                m_new = jnp.maximum(m_prev, jnp.max(sc, axis=1, keepdims=True))
                p = jnp.exp2(sc - m_new[:, :1])
                alpha = jnp.exp2(m_prev - m_new)
                l_ref[rows, :] = alpha * l_ref[rows, :] + jnp.sum(p, axis=1, keepdims=True)
                m_ref[rows, :] = m_new
                pv = jnp.dot(p.astype(BF16), c, preferred_element_type=F32)
                acc_ref[rows, :] = acc_ref[rows, :] * alpha[:, :1] + pv

        pc = acc_ref[...] / l_ref[...][:, :1]
        lane = lax.broadcasted_iota(jnp.int32, (64, 128), 1)
        row = lax.broadcasted_iota(jnp.int32, (64, 128), 0)
        dmask = (lane % 32) == (row % 32)
        ctx = jnp.zeros((64, D), F32)
        for j in range(4):
            pcj = pc[:, j * 128:(j + 1) * 128]
            for t in range(32):
                gth = jnp.take_along_axis(pcj, lane // 32 + 4 * t, axis=1)
                a_buf[:, t * 128:(t + 1) * 128] = jnp.where(dmask, gth, 0.0).astype(BF16)
            wait(i_wuv[j])
            v2 = wuv_buf[pl.ds(j * 128, 128)].reshape(4096, D)
            ctx = ctx + jnp.dot(a_buf[...], v2, preferred_element_type=F32)

        hrow = row % 32
        r = jnp.zeros((64, M), F32)
        for j in range(4):
            for t in range(8):
                h = j * 8 + t
                a_buf[:, t * 128:(t + 1) * 128] = jnp.where(hrow == h, ctx, 0.0).astype(BF16)
            wait(i_wo[j])
            o2 = wo_buf[pl.ds(j * 8, 8)].reshape(1024, M)
            r = r + jnp.dot(a_buf[:, 0:1024], o2, preferred_element_type=F32)
        s0 = jnp.sum(r[0:32], axis=0, keepdims=True)
        s1 = jnp.sum(r[32:64], axis=0, keepdims=True)
        s = jnp.concatenate([s0, s1], axis=0)

        small[1].wait(); small[2].wait()
        hacc = jnp.zeros((B, F), F32)
        for j in range(2):
            wait(i_w1[j])
            hacc = hacc + jnp.dot(xn_b[:, j * 256:(j + 1) * 256], w1_buf[pl.ds(j * 256, 256), :], preferred_element_type=F32)
        hh = hacc + b1_buf[...].astype(F32).reshape(1, F)
        hh = jax.nn.gelu(hh, approximate=True).astype(BF16)
        gacc = jnp.zeros((B, M), F32)
        for j in range(7):
            wait(i_w2[j])
            gacc = gacc + jnp.dot(hh[:, j * 256:(j + 1) * 256], w2_buf[pl.ds(j * 256, 256), :], preferred_element_type=F32)
        gg = gacc + b2_buf[...].astype(F32).reshape(1, M)
        g = gg * jax.nn.sigmoid(gg)
        o_ref[...] = (x + s * g).astype(BF16)

    ncop = 4 + 4 + 2 * NKB + 4 + 4 + 2 + 7

    def fn(A_x, A_c_kv, A_w_q, A_w_uk, A_w_uv, A_w_o, B_x, B_w1, B_b1, B_w2, B_b2):
        del B_x
        return pl.pallas_call(
            kernel,
            out_shape=jax.ShapeDtypeStruct((B, M), BF16),
            in_specs=[pl.BlockSpec(memory_space=pltpu.HBM)] * 10,
            out_specs=pl.BlockSpec(memory_space=pltpu.VMEM),
            scratch_shapes=[
                pltpu.VMEM((B, M), BF16), pltpu.VMEM((F,), BF16), pltpu.VMEM((M,), BF16),
                pltpu.VMEM((B, SK, DC), BF16),
                pltpu.VMEM((M, H, D), BF16), pltpu.VMEM((DC, H, D), BF16), pltpu.VMEM((DC, H, D), BF16),
                pltpu.VMEM((H, D, M), BF16), pltpu.VMEM((M, F), BF16), pltpu.VMEM((F, M), BF16),
                pltpu.VMEM((B, M), F32), pltpu.SMEM((B, M), F32),
                pltpu.VMEM((DC * 8, 128), F32),
                pltpu.VMEM((B * H, DC), BF16), pltpu.VMEM((B * H, DC), F32),
                pltpu.VMEM((B * H, 128), F32), pltpu.VMEM((B * H, 128), F32),
                pltpu.VMEM((64, 4096), BF16),
                pltpu.SemaphoreType.DMA((ncop,)), pltpu.SemaphoreType.DMA((4,)),
            ],
            compiler_params=pltpu.CompilerParams(vmem_limit_bytes=100 * 1024 * 1024),
        )(A_x.reshape(B, M), A_c_kv, A_w_q, A_w_uk, A_w_uv, A_w_o, B_w1, B_b1, B_w2, B_b2).reshape(B, 1, M)
    return fn


_impl = make_kernel()


@jax.jit
def pallas_recurrent_scan__compressed_kv_cla__dense_activation_gelu__decode_kernel(
    A_x: jax.Array,
    A_c_kv: jax.Array,
    A_w_q: jax.Array,
    A_w_uk: jax.Array,
    A_w_uv: jax.Array,
    A_w_o: jax.Array,
    B_x: jax.Array,
    B_w1: jax.Array,
    B_b1: jax.Array,
    B_w2: jax.Array,
    B_b2: jax.Array,
):
    return _impl(A_x, A_c_kv, A_w_q, A_w_uk, A_w_uv, A_w_o, B_x, B_w1, B_b1, B_w2, B_b2)
```

```python
import functools
import jax
import jax.numpy as jnp
import numpy as np
from jax import lax
import jax.experimental.pallas as pl
import jax.experimental.pallas.tpu as pltpu

F32 = jnp.float32
BF16 = jnp.bfloat16

B, H, SK, D, M, DC, F = 2, 32, 16384, 128, 512, 512, 1792
LOG2E = 1.4426950408889634


def make_kernel(BK=2048, CK=4096, AHEAD=3, UNROLL_Q=8, W2S=(1024, 512, 256), PRIO=True, TANH=True, NSEM=None, W1POS='late'):
    NCK = SK // CK
    NC = B * NCK
    W2O = [sum(W2S[:i]) for i in range(len(W2S))]
    assert sum(W2S) == F
    NSEM = NSEM or AHEAD

    def kernel(x_hbm, ckv_hbm, wq_hbm, wuk_hbm, wuv_hbm, wo_hbm, w1_hbm, b1_hbm, w2_hbm, b2_hbm,
               o_ref,
               x_buf, b1_buf, b2_buf, c_buf, wq_buf, wuk_buf, wuv_buf, wo_buf, w1_buf, w2_buf,
               xn_v, xs, t8, qa_ref, acc_ref, m_ref, l_ref, a_buf, sems, sem_small):
        def rows(hbm, buf, o, n):
            return (hbm.at[pl.ds(o, n)], buf.at[pl.ds(o, n)])
        pre = [rows(wq_hbm, wq_buf, 0, 256), rows(wq_hbm, wq_buf, 256, 256),
               rows(wuk_hbm, wuk_buf, 0, 256), rows(wuk_hbm, wuk_buf, 256, 256)]
        post = [rows(wuv_hbm, wuv_buf, 0, 256), rows(wuv_hbm, wuv_buf, 256, 256),
                rows(wo_hbm, wo_buf, 0, 16), rows(wo_hbm, wo_buf, 16, 16),
                (w1_hbm, w1_buf)] + [rows(w2_hbm, w2_buf, o, n) for o, n in zip(W2O, W2S)]
        NPRE = len(pre)
        ncop = NPRE + NC + len(post)

        def ckv_pair(ci):
            b = ci // NCK
            o = (ci % NCK) * CK
            if not isinstance(ci, int):
                o = pl.multiple_of(o, CK)
            return (ckv_hbm.at[b, pl.ds(o, CK)], c_buf.at[b, pl.ds(o, CK)])

        def static_copy(i):
            if i < NPRE:
                s, d = pre[i]
            elif i < NPRE + NC:
                s, d = ckv_pair(i - NPRE)
            else:
                s, d = post[i - NPRE - NC]
            return pltpu.make_async_copy(s, d, sems.at[i % NSEM])

        def start(i):
            if i < ncop:
                static_copy(i).start(priority=(i % 2) if PRIO else 0)

        def wait(i):
            static_copy(i).wait()
            start(i + AHEAD)

        small = [pltpu.make_async_copy(x_hbm, x_buf, sem_small.at[0]),
                 pltpu.make_async_copy(b1_hbm, b1_buf, sem_small.at[1]),
                 pltpu.make_async_copy(b2_hbm, b2_buf, sem_small.at[1])]
        start(0)
        small[0].start()
        for i in range(1, AHEAD):
            start(i)
        small[1].start(); small[2].start()

        small[0].wait()
        x = x_buf[...].astype(F32)
        mu = jnp.mean(x, axis=-1, keepdims=True)
        xc = x - mu
        var = jnp.mean(xc * xc, axis=-1, keepdims=True)
        xn = xc * lax.rsqrt(var + 1e-5)
        xn_b = xn.astype(BF16)
        xn_v[...] = xn_b.astype(F32)
        cp = pltpu.make_async_copy(xn_v, xs, sem_small.at[0])
        cp.start(); cp.wait()

        carry = (jnp.zeros((H, D), F32), jnp.zeros((H, D), F32))
        for j in range(2):
            wait(j)
            def body(i, carry, j=j):
                a0, a1 = carry
                for u in range(UNROLL_Q):
                    m = j * 256 + i * UNROLL_Q + u
                    w = wq_buf[m].astype(F32)
                    a0 = a0 + xs[0, m] * w
                    a1 = a1 + xs[1, m] * w
                return a0, a1
            carry = lax.fori_loop(0, 256 // UNROLL_Q, body, carry)
        q = jnp.concatenate([carry[0], carry[1], jnp.zeros((64, D), F32)], axis=0).astype(BF16)

        lane3 = lax.broadcasted_iota(jnp.int32, (16, 8, 128), 2)
        g3 = (lane3 % 32) // 8
        for j in range(2):
            wait(2 + j)
            def body(s, _, j=j):
                c0 = pl.multiple_of(j * 256 + s * 16, 16)
                u = wuk_buf[pl.ds(c0, 16)].reshape(16 * 32, D)
                r = lax.dot_general(u, q, (((1,), (1,)), ((), ())), preferred_element_type=F32)
                r4 = r.reshape(16, 4, 8, 128)
                v = jnp.where(g3 == 0, r4[:, 0], jnp.where(g3 == 1, r4[:, 1], jnp.where(g3 == 2, r4[:, 2], r4[:, 3])))
                t8[pl.ds(pl.multiple_of(c0 * 8, 128), 128), :] = v.reshape(128, 128)
            lax.fori_loop(0, 16, body, None, unroll=2)
        lane2 = lax.broadcasted_iota(jnp.int32, (128, 128), 1) % 8
        scale = (D ** -0.5) * LOG2E
        for j in range(4):
            t = t8[pl.ds(j * 1024, 128, stride=8), :]
            for s in range(1, 8):
                t = jnp.where(lane2 == s, t8[pl.ds(j * 1024 + s, 128, stride=8), :], t)
            tt = t.T
            qa_ref[:, j * 128:(j + 1) * 128] = (tt[:64] * scale).astype(BF16)

        m_ref[...] = jnp.full((B * H, 128), -1e30, F32)
        l_ref[...] = jnp.zeros((B * H, 128), F32)
        acc_ref[...] = jnp.zeros((B * H, DC), F32)

        def chunk(ci, _):
            i = NPRE + ci
            s, d = ckv_pair(ci)
            pltpu.make_async_copy(s, d, sems.at[i % NSEM]).wait()
            nxt = ci + AHEAD

            @pl.when(nxt < NC)
            def _():
                s2, d2 = ckv_pair(nxt)
                cpn = pltpu.make_async_copy(s2, d2, sems.at[(i + AHEAD) % NSEM])
                if PRIO:
                    @pl.when(nxt % 2 == 0)
                    def _():
                        cpn.start(priority=NPRE % 2)
                    @pl.when(nxt % 2 == 1)
                    def _():
                        cpn.start(priority=(NPRE + 1) % 2)
                else:
                    cpn.start()
            for e in range(AHEAD):
                @pl.when(nxt == NC + e)
                def _(e=e):
                    start(NPRE + NC + e)

            b = ci // NCK
            hrows = pl.ds(pl.multiple_of(b * H, H), H)

            def block(jj, _):
                o = pl.multiple_of((ci % NCK) * CK + jj * BK, BK)
                qa = qa_ref[hrows, :]
                c = c_buf[b, pl.ds(o, BK), :]
                sc = lax.dot_general(qa, c, (((1,), (1,)), ((), ())), preferred_element_type=F32)
                m_prev = m_ref[hrows, :]
                m_new = jnp.maximum(m_prev, jnp.max(sc, axis=1, keepdims=True))
                p = jnp.exp2(sc - m_new[:, :1])
                alpha = jnp.exp2(m_prev - m_new)
                l_ref[hrows, :] = alpha * l_ref[hrows, :] + jnp.sum(p, axis=1, keepdims=True)
                m_ref[hrows, :] = m_new
                pv = jnp.dot(p.astype(BF16), c, preferred_element_type=F32)
                acc_ref[hrows, :] = acc_ref[hrows, :] * alpha[:, :1] + pv
            lax.fori_loop(0, CK // BK, block, None)
        lax.fori_loop(0, NC, chunk, None)

        pc = acc_ref[...] / l_ref[...][:, :1]
        lane = lax.broadcasted_iota(jnp.int32, (64, 128), 1)
        row = lax.broadcasted_iota(jnp.int32, (64, 128), 0)
        dmask = (lane % 32) == (row % 32)
        ctx = jnp.zeros((64, D), F32)
        for j in range(4):
            pcj = pc[:, j * 128:(j + 1) * 128]
            for t in range(32):
                gth = jnp.take_along_axis(pcj, lane // 32 + 4 * t, axis=1)
                a_buf[:, t * 128:(t + 1) * 128] = jnp.where(dmask, gth, 0.0).astype(BF16)
            if j % 2 == 0:
                wait(NPRE + NC + j // 2)
            v2 = wuv_buf[pl.ds(j * 128, 128)].reshape(4096, D)
            ctx = ctx + jnp.dot(a_buf[...], v2, preferred_element_type=F32)

        hrow = row % 32
        r = jnp.zeros((64, M), F32)
        for j in range(4):
            for t in range(8):
                h = j * 8 + t
                a_buf[:, t * 128:(t + 1) * 128] = jnp.where(hrow == h, ctx, 0.0).astype(BF16)
            if j % 2 == 0:
                wait(NPRE + NC + 2 + j // 2)
            o2 = wo_buf[pl.ds(j * 8, 8)].reshape(1024, M)
            r = r + jnp.dot(a_buf[:, 0:1024], o2, preferred_element_type=F32)
        s0 = jnp.sum(r[0:32], axis=0, keepdims=True)
        s1 = jnp.sum(r[32:64], axis=0, keepdims=True)
        s = jnp.concatenate([s0, s1], axis=0)

        small[1].wait(); small[2].wait()
        wait(NPRE + NC + 4)
        hacc = jnp.dot(xn_b, w1_buf[...], preferred_element_type=F32)
        hh = hacc + b1_buf[...].astype(F32).reshape(1, F)
        hh = jax.nn.gelu(hh, approximate=True).astype(BF16)
        gg = b2_buf[...].astype(F32).reshape(1, M)
        for j, (o, n) in enumerate(zip(W2O, W2S)):
            wait(NPRE + NC + 5 + j)
            gg = gg + jnp.dot(hh[:, o:o + n], w2_buf[pl.ds(o, n), :], preferred_element_type=F32)
        if TANH:
            hg = 0.5 * gg
            g = hg * jnp.tanh(hg) + hg
        else:
            g = gg * jax.nn.sigmoid(gg)
        o_ref[...] = (x + s * g).astype(BF16)

    def fn(A_x, A_c_kv, A_w_q, A_w_uk, A_w_uv, A_w_o, B_x, B_w1, B_b1, B_w2, B_b2):
        del B_x
        return pl.pallas_call(
            kernel,
            out_shape=jax.ShapeDtypeStruct((B, M), BF16),
            in_specs=[pl.BlockSpec(memory_space=pltpu.HBM)] * 10,
            out_specs=pl.BlockSpec(memory_space=pltpu.VMEM),
            scratch_shapes=[
                pltpu.VMEM((B, M), BF16), pltpu.VMEM((F,), BF16), pltpu.VMEM((M,), BF16),
                pltpu.VMEM((B, SK, DC), BF16),
                pltpu.VMEM((M, H, D), BF16), pltpu.VMEM((DC, H, D), BF16), pltpu.VMEM((DC, H, D), BF16),
                pltpu.VMEM((H, D, M), BF16), pltpu.VMEM((M, F), BF16), pltpu.VMEM((F, M), BF16),
                pltpu.VMEM((B, M), F32), pltpu.SMEM((B, M), F32),
                pltpu.VMEM((DC * 8, 128), F32),
                pltpu.VMEM((B * H, DC), BF16), pltpu.VMEM((B * H, DC), F32),
                pltpu.VMEM((B * H, 128), F32), pltpu.VMEM((B * H, 128), F32),
                pltpu.VMEM((64, 4096), BF16),
                pltpu.SemaphoreType.DMA((NSEM,)), pltpu.SemaphoreType.DMA((2,)),
            ],
            compiler_params=pltpu.CompilerParams(vmem_limit_bytes=100 * 1024 * 1024),
        )(A_x.reshape(B, M), A_c_kv, A_w_q, A_w_uk, A_w_uv, A_w_o, B_w1, B_b1, B_w2, B_b2).reshape(B, 1, M)
    return fn


_impl = make_kernel()


@jax.jit
def pallas_recurrent_scan__compressed_kv_cla__dense_activation_gelu__decode_kernel(
    A_x: jax.Array,
    A_c_kv: jax.Array,
    A_w_q: jax.Array,
    A_w_uk: jax.Array,
    A_w_uv: jax.Array,
    A_w_o: jax.Array,
    B_x: jax.Array,
    B_w1: jax.Array,
    B_b1: jax.Array,
    B_w2: jax.Array,
    B_b2: jax.Array,
):
    return _impl(A_x, A_c_kv, A_w_q, A_w_uk, A_w_uv, A_w_o, B_x, B_w1, B_b1, B_w2, B_b2)
```

```python
import jax
import jax.numpy as jnp
from jax import lax
import jax.experimental.pallas as pl
import jax.experimental.pallas.tpu as pltpu

F32 = jnp.float32
BF16 = jnp.bfloat16

B, H, SK, D, M, DC, F = 2, 32, 16384, 128, 512, 512, 1792
LOG2E = 1.4426950408889634

CK = 4096
BK = 2048
NCK = SK // CK
NC = B * NCK
AHEAD = 3
W2_ROWS = (1280, 384, 128)
NT = (((1,), (1,)), ((), ()))


def _kernel(x_hbm, ckv_hbm, wq_hbm, wuk_hbm, wuv_hbm, wo_hbm, w1_hbm, b1_hbm, w2_hbm, b2_hbm,
            o_ref,
            x_buf, b1_buf, b2_buf, c_buf, wq_buf, wuk_buf, wuv_buf, wo_buf, w1_buf, w2_buf,
            xn_vmem, xn_smem, t8, qa_ref, acc_ref, m_ref, l_ref, a_buf, sems, sem_small):
    def rows(hbm, buf, o, n):
        return hbm.at[pl.ds(o, n)], buf.at[pl.ds(o, n)]

    w2_off = [sum(W2_ROWS[:i]) for i in range(len(W2_ROWS))]
    pre = [rows(wq_hbm, wq_buf, 0, M // 2), rows(wq_hbm, wq_buf, M // 2, M // 2),
           rows(wuk_hbm, wuk_buf, 0, DC // 2), rows(wuk_hbm, wuk_buf, DC // 2, DC // 2)]
    post = [rows(wuv_hbm, wuv_buf, 0, DC // 2), rows(wuv_hbm, wuv_buf, DC // 2, DC // 2),
            rows(wo_hbm, wo_buf, 0, H // 2), rows(wo_hbm, wo_buf, H // 2, H // 2),
            (w1_hbm, w1_buf)] + [rows(w2_hbm, w2_buf, o, n) for o, n in zip(w2_off, W2_ROWS)]
    n_pre = len(pre)
    i_post = n_pre + NC
    n_copies = i_post + len(post)

    def ckv_pair(ci):
        b, o = ci // NCK, (ci % NCK) * CK
        if not isinstance(ci, int):
            o = pl.multiple_of(o, CK)
        return ckv_hbm.at[b, pl.ds(o, CK)], c_buf.at[b, pl.ds(o, CK)]

    def copy(i):
        src, dst = pre[i] if i < n_pre else ckv_pair(i - n_pre) if i < i_post else post[i - i_post]
        return pltpu.make_async_copy(src, dst, sems.at[i % AHEAD])

    def start(i):
        if i < n_copies:
            copy(i).start()

    def wait(i):
        copy(i).wait()
        start(i + AHEAD)

    x_copy = pltpu.make_async_copy(x_hbm, x_buf, sem_small.at[0])
    b1_copy = pltpu.make_async_copy(b1_hbm, b1_buf, sem_small.at[1])
    b2_copy = pltpu.make_async_copy(b2_hbm, b2_buf, sem_small.at[1])
    start(0)
    x_copy.start()
    for i in range(1, AHEAD):
        start(i)
    b1_copy.start()
    b2_copy.start()

    x_copy.wait()
    x = x_buf[...].astype(F32)
    xc = x - jnp.mean(x, axis=-1, keepdims=True)
    var = jnp.mean(xc * xc, axis=-1, keepdims=True)
    xn = (xc * lax.rsqrt(var + 1e-5)).astype(BF16)
    xn_vmem[...] = xn.astype(F32)
    to_smem = pltpu.make_async_copy(xn_vmem, xn_smem, sem_small.at[0])
    to_smem.start()
    to_smem.wait()

    unroll = 8
    q01 = (jnp.zeros((H, D), F32), jnp.zeros((H, D), F32))
    for j in range(2):
        wait(j)

        def q_body(i, carry, j=j):
            q0, q1 = carry
            for u in range(unroll):
                m = j * (M // 2) + i * unroll + u
                w = wq_buf[m].astype(F32)
                q0 = q0 + xn_smem[0, m] * w
                q1 = q1 + xn_smem[1, m] * w
            return q0, q1

        q01 = lax.fori_loop(0, M // 2 // unroll, q_body, q01)
    q = jnp.concatenate([q01[0], q01[1], jnp.zeros((128 - B * H, D), F32)], axis=0).astype(BF16)

    group = (lax.broadcasted_iota(jnp.int32, (16, 8, 128), 2) % H) // 8
    for j in range(2):
        wait(2 + j)

        def qa_body(s, _, j=j):
            c0 = pl.multiple_of(j * (DC // 2) + s * 16, 16)
            u = wuk_buf[pl.ds(c0, 16)].reshape(16 * H, D)
            r = lax.dot_general(u, q, NT, preferred_element_type=F32).reshape(16, 4, 8, 128)
            v = jnp.where(group == 0, r[:, 0],
                          jnp.where(group == 1, r[:, 1], jnp.where(group == 2, r[:, 2], r[:, 3])))
            t8[pl.ds(pl.multiple_of(c0 * 8, 128), 128), :] = v.reshape(128, 128)

        lax.fori_loop(0, DC // 2 // 16, qa_body, None, unroll=2)
    sub = lax.broadcasted_iota(jnp.int32, (128, 128), 1) % 8
    for j in range(DC // 128):
        t = t8[pl.ds(j * 1024, 128, stride=8), :]
        for s in range(1, 8):
            t = jnp.where(sub == s, t8[pl.ds(j * 1024 + s, 128, stride=8), :], t)
        qa_ref[:, j * 128:(j + 1) * 128] = (t.T[:B * H] * (D ** -0.5 * LOG2E)).astype(BF16)

    m_ref[...] = jnp.full((B * H, 128), -1e30, F32)
    l_ref[...] = jnp.zeros((B * H, 128), F32)
    acc_ref[...] = jnp.zeros((B * H, DC), F32)

    def chunk(ci, _):
        i = n_pre + ci
        pltpu.make_async_copy(*ckv_pair(ci), sems.at[i % AHEAD]).wait()
        nxt = ci + AHEAD

        @pl.when(nxt < NC)
        def _():
            pltpu.make_async_copy(*ckv_pair(nxt), sems.at[(i + AHEAD) % AHEAD]).start()

        for e in range(AHEAD):
            pl.when(nxt == NC + e)(lambda e=e: start(i_post + e))

        b = ci // NCK
        hrows = pl.ds(pl.multiple_of(b * H, H), H)

        def block(jj, _):
            o = pl.multiple_of((ci % NCK) * CK + jj * BK, BK)
            c = c_buf[b, pl.ds(o, BK), :]
            sc = lax.dot_general(qa_ref[hrows, :], c, NT, preferred_element_type=F32)
            m_prev = m_ref[hrows, :]
            m_new = jnp.maximum(m_prev, jnp.max(sc, axis=1, keepdims=True))
            p = jnp.exp2(sc - m_new[:, :1])
            alpha = jnp.exp2(m_prev - m_new)
            l_ref[hrows, :] = alpha * l_ref[hrows, :] + jnp.sum(p, axis=1, keepdims=True)
            m_ref[hrows, :] = m_new
            pv = jnp.dot(p.astype(BF16), c, preferred_element_type=F32)
            acc_ref[hrows, :] = acc_ref[hrows, :] * alpha[:, :1] + pv

        lax.fori_loop(0, CK // BK, block, None)

    lax.fori_loop(0, NC, chunk, None)

    pc = acc_ref[...] / l_ref[...][:, :1]
    lane = lax.broadcasted_iota(jnp.int32, (B * H, 128), 1)
    head = lax.broadcasted_iota(jnp.int32, (B * H, 128), 0) % H
    diag = (lane % H) == head
    ctx = jnp.zeros((B * H, D), F32)
    for j in range(DC // 128):
        pcj = pc[:, j * 128:(j + 1) * 128]
        for t in range(32):
            rep = jnp.take_along_axis(pcj, lane // H + 4 * t, axis=1)
            a_buf[:, t * 128:(t + 1) * 128] = jnp.where(diag, rep, 0.0).astype(BF16)
        if j % 2 == 0:
            wait(i_post + j // 2)
        v2 = wuv_buf[pl.ds(j * 128, 128)].reshape(128 * H, D)
        ctx = ctx + jnp.dot(a_buf[...], v2, preferred_element_type=F32)

    r = jnp.zeros((B * H, M), F32)
    for j in range(4):
        for t in range(8):
            a_buf[:, t * 128:(t + 1) * 128] = jnp.where(head == j * 8 + t, ctx, 0.0).astype(BF16)
        if j % 2 == 0:
            wait(i_post + 2 + j // 2)
        o2 = wo_buf[pl.ds(j * 8, 8)].reshape(8 * D, M)
        r = r + jnp.dot(a_buf[:, 0:8 * D], o2, preferred_element_type=F32)
    s = jnp.concatenate([jnp.sum(r[b * H:(b + 1) * H], axis=0, keepdims=True) for b in range(B)], axis=0)

    b1_copy.wait()
    b2_copy.wait()
    wait(i_post + 4)
    h = jnp.dot(xn, w1_buf[...], preferred_element_type=F32) + b1_buf[...].astype(F32).reshape(1, F)
    h = jax.nn.gelu(h, approximate=True).astype(BF16)
    gg = b2_buf[...].astype(F32).reshape(1, M)
    for j, (o, n) in enumerate(zip(w2_off, W2_ROWS)):
        wait(i_post + 5 + j)
        gg = gg + jnp.dot(h[:, o:o + n], w2_buf[pl.ds(o, n), :], preferred_element_type=F32)
    half = 0.5 * gg
    gate = half * jnp.tanh(half) + half
    o_ref[...] = (x + s * gate).astype(BF16)


@jax.jit
def pallas_recurrent_scan__compressed_kv_cla__dense_activation_gelu__decode_kernel(
    A_x: jax.Array,
    A_c_kv: jax.Array,
    A_w_q: jax.Array,
    A_w_uk: jax.Array,
    A_w_uv: jax.Array,
    A_w_o: jax.Array,
    B_x: jax.Array,
    B_w1: jax.Array,
    B_b1: jax.Array,
    B_w2: jax.Array,
    B_b2: jax.Array,
):
    del B_x
    out = pl.pallas_call(
        _kernel,
        out_shape=jax.ShapeDtypeStruct((B, M), BF16),
        in_specs=[pl.BlockSpec(memory_space=pltpu.HBM)] * 10,
        out_specs=pl.BlockSpec(memory_space=pltpu.VMEM),
        scratch_shapes=[
            pltpu.VMEM((B, M), BF16), pltpu.VMEM((F,), BF16), pltpu.VMEM((M,), BF16),
            pltpu.VMEM((B, SK, DC), BF16),
            pltpu.VMEM((M, H, D), BF16), pltpu.VMEM((DC, H, D), BF16), pltpu.VMEM((DC, H, D), BF16),
            pltpu.VMEM((H, D, M), BF16), pltpu.VMEM((M, F), BF16), pltpu.VMEM((F, M), BF16),
            pltpu.VMEM((B, M), F32), pltpu.SMEM((B, M), F32),
            pltpu.VMEM((DC * 8 + 8, 128), F32),
            pltpu.VMEM((B * H, DC), BF16), pltpu.VMEM((B * H, DC), F32),
            pltpu.VMEM((B * H, 128), F32), pltpu.VMEM((B * H, 128), F32),
            pltpu.VMEM((B * H, 128 * H), BF16),
            pltpu.SemaphoreType.DMA((AHEAD,)), pltpu.SemaphoreType.DMA((2,)),
        ],
        compiler_params=pltpu.CompilerParams(vmem_limit_bytes=100 * 1024 * 1024),
    )(A_x.reshape(B, M), A_c_kv, A_w_q, A_w_uk, A_w_uv, A_w_o, B_w1, B_b1, B_w2, B_b2)
    return out.reshape(B, 1, M)
```

```python
import jax
import jax.numpy as jnp
from jax import lax
import jax.experimental.pallas as pl
import jax.experimental.pallas.tpu as pltpu

F32 = jnp.float32
BF16 = jnp.bfloat16

B, H, SK, D, M, DC, F = 2, 32, 16384, 128, 512, 512, 1792
LOG2E = 1.4426950408889634

CK = 4096
BK = 2048
NCK = SK // CK
NC = B * NCK
AHEAD = 3
W2_ROWS = (1280, 384, 128)
NT = (((1,), (1,)), ((), ()))


def _kernel(x_hbm, ckv_hbm, wq_hbm, wuk_hbm, wuv_hbm, wo_hbm, w1_hbm, b1_hbm, w2_hbm, b2_hbm,
            o_ref,
            x_buf, b1_buf, b2_buf, c_buf, wq_buf, wuk_buf, wuv_buf, wo_buf, w1_buf, w2_buf,
            xn_vmem, xn_smem, t8, qa_ref, acc_ref, m_ref, l_ref, a_buf, sems, sem_small):
    def rows(hbm, buf, o, n):
        return hbm.at[pl.ds(o, n)], buf.at[pl.ds(o, n)]

    w2_off = [sum(W2_ROWS[:i]) for i in range(len(W2_ROWS))]
    pre = [rows(wq_hbm, wq_buf, 0, M // 2), rows(wq_hbm, wq_buf, M // 2, M // 2),
           rows(wuk_hbm, wuk_buf, 0, DC // 2), rows(wuk_hbm, wuk_buf, DC // 2, DC // 2)]
    post = [rows(wuv_hbm, wuv_buf, 0, DC // 2), rows(wuv_hbm, wuv_buf, DC // 2, DC // 2),
            rows(wo_hbm, wo_buf, 0, H // 2), rows(wo_hbm, wo_buf, H // 2, H // 2),
            (w1_hbm, w1_buf)] + [rows(w2_hbm, w2_buf, o, n) for o, n in zip(w2_off, W2_ROWS)]
    n_pre = len(pre)
    i_post = n_pre + NC
    n_copies = i_post + len(post)

    def ckv_pair(ci):
        b, o = ci // NCK, (ci % NCK) * CK
        if not isinstance(ci, int):
            o = pl.multiple_of(o, CK)
        return ckv_hbm.at[b, pl.ds(o, CK)], c_buf.at[b, pl.ds(o, CK)]

    def copy(i):
        src, dst = pre[i] if i < n_pre else ckv_pair(i - n_pre) if i < i_post else post[i - i_post]
        return pltpu.make_async_copy(src, dst, sems.at[i % AHEAD])

    def start(i):
        if i < n_copies:
            copy(i).start()

    def wait(i):
        copy(i).wait()
        start(i + AHEAD)

    x_copy = pltpu.make_async_copy(x_hbm, x_buf, sem_small.at[0])
    b1_copy = pltpu.make_async_copy(b1_hbm, b1_buf, sem_small.at[1])
    b2_copy = pltpu.make_async_copy(b2_hbm, b2_buf, sem_small.at[1])
    start(0)
    x_copy.start()
    for i in range(1, AHEAD):
        start(i)
    b1_copy.start()
    b2_copy.start()

    x_copy.wait()
    x = x_buf[...].astype(F32)
    xc = x - jnp.mean(x, axis=-1, keepdims=True)
    var = jnp.mean(xc * xc, axis=-1, keepdims=True)
    xn = (xc * lax.rsqrt(var + 1e-5)).astype(BF16)
    xn_vmem[...] = xn.astype(F32)
    to_smem = pltpu.make_async_copy(xn_vmem, xn_smem, sem_small.at[0])
    to_smem.start()
    to_smem.wait()

    unroll = 8
    q01 = (jnp.zeros((H, D), F32), jnp.zeros((H, D), F32))
    for j in range(2):
        wait(j)

        def q_body(i, carry, j=j):
            q0, q1 = carry
            for u in range(unroll):
                m = j * (M // 2) + i * unroll + u
                w = wq_buf[m].astype(F32)
                q0 = q0 + xn_smem[0, m] * w
                q1 = q1 + xn_smem[1, m] * w
            return q0, q1

        q01 = lax.fori_loop(0, M // 2 // unroll, q_body, q01)
    q = jnp.concatenate([q01[0], q01[1], jnp.zeros((128 - B * H, D), F32)], axis=0).astype(BF16)

    group = (lax.broadcasted_iota(jnp.int32, (16, 8, 128), 2) % H) // 8
    for j in range(2):
        wait(2 + j)

        def qa_body(s, _, j=j):
            c0 = pl.multiple_of(j * (DC // 2) + s * 16, 16)
            u = wuk_buf[pl.ds(c0, 16)].reshape(16 * H, D)
            r = lax.dot_general(u, q, NT, preferred_element_type=F32).reshape(16, 4, 8, 128)
            v = jnp.where(group == 0, r[:, 0],
                          jnp.where(group == 1, r[:, 1], jnp.where(group == 2, r[:, 2], r[:, 3])))
            t8[pl.ds(pl.multiple_of(c0 * 8, 128), 128), :] = v.reshape(128, 128)

        lax.fori_loop(0, DC // 2 // 16, qa_body, None, unroll=2)
    sub = lax.broadcasted_iota(jnp.int32, (128, 128), 1) % 8
    for j in range(DC // 128):
        t = t8[pl.ds(j * 1024, 128, stride=8), :]
        for s in range(1, 8):
            t = jnp.where(sub == s, t8[pl.ds(j * 1024 + s, 128, stride=8), :], t)
        qa_ref[:, j * 128:(j + 1) * 128] = (t.T[:B * H] * (D ** -0.5 * LOG2E)).astype(BF16)

    m_ref[...] = jnp.full((B * H, 128), -jnp.inf, F32)
    l_ref[...] = jnp.zeros((B * H, 128), F32)
    acc_ref[...] = jnp.zeros((B * H, DC), F32)

    def chunk(ci, _):
        i = n_pre + ci
        pltpu.make_async_copy(*ckv_pair(ci), sems.at[i % AHEAD]).wait()
        nxt = ci + AHEAD

        @pl.when(nxt < NC)
        def _():
            pltpu.make_async_copy(*ckv_pair(nxt), sems.at[(i + AHEAD) % AHEAD]).start()

        for e in range(AHEAD):
            pl.when(nxt == NC + e)(lambda e=e: start(i_post + e))

        b = ci // NCK
        hrows = pl.ds(pl.multiple_of(b * H, H), H)

        def block(jj, _):
            o = pl.multiple_of((ci % NCK) * CK + jj * BK, BK)
            c = c_buf[b, pl.ds(o, BK), :]
            sc = lax.dot_general(qa_ref[hrows, :], c, NT, preferred_element_type=F32)
            m_prev = m_ref[hrows, :]
            m_new = jnp.maximum(m_prev, jnp.max(sc, axis=1, keepdims=True))
            p = jnp.exp2(sc - m_new[:, :1])
            alpha = jnp.exp2(m_prev - m_new)
            l_ref[hrows, :] = alpha * l_ref[hrows, :] + jnp.sum(p, axis=1, keepdims=True)
            m_ref[hrows, :] = m_new
            pv = jnp.dot(p.astype(BF16), c, preferred_element_type=F32)
            acc_ref[hrows, :] = acc_ref[hrows, :] * alpha[:, :1] + pv

        lax.fori_loop(0, CK // BK, block, None)

    lax.fori_loop(0, NC, chunk, None)

    pc = acc_ref[...] / l_ref[...][:, :1]
    lane = lax.broadcasted_iota(jnp.int32, (B * H, 128), 1)
    head = lax.broadcasted_iota(jnp.int32, (B * H, 128), 0) % H
    diag = (lane % H) == head
    ctx = jnp.zeros((B * H, D), F32)
    for j in range(DC // 128):
        pcj = pc[:, j * 128:(j + 1) * 128]
        for t in range(32):
            rep = jnp.take_along_axis(pcj, lane // H + 4 * t, axis=1)
            a_buf[:, t * 128:(t + 1) * 128] = jnp.where(diag, rep, 0.0).astype(BF16)
        if j % 2 == 0:
            wait(i_post + j // 2)
        v2 = wuv_buf[pl.ds(j * 128, 128)].reshape(128 * H, D)
        ctx = ctx + jnp.dot(a_buf[...], v2, preferred_element_type=F32)

    r = jnp.zeros((B * H, M), F32)
    for j in range(4):
        for t in range(8):
            a_buf[:, t * 128:(t + 1) * 128] = jnp.where(head == j * 8 + t, ctx, 0.0).astype(BF16)
        if j % 2 == 0:
            wait(i_post + 2 + j // 2)
        o2 = wo_buf[pl.ds(j * 8, 8)].reshape(8 * D, M)
        r = r + jnp.dot(a_buf[:, 0:8 * D], o2, preferred_element_type=F32)
    s = jnp.concatenate([jnp.sum(r[b * H:(b + 1) * H], axis=0, keepdims=True) for b in range(B)], axis=0)

    b1_copy.wait()
    b2_copy.wait()
    wait(i_post + 4)
    h = jnp.dot(xn, w1_buf[...], preferred_element_type=F32) + b1_buf[...].astype(F32).reshape(1, F)
    h = jax.nn.gelu(h, approximate=True).astype(BF16)
    gg = b2_buf[...].astype(F32).reshape(1, M)
    for j, (o, n) in enumerate(zip(w2_off, W2_ROWS)):
        wait(i_post + 5 + j)
        gg = gg + jnp.dot(h[:, o:o + n], w2_buf[pl.ds(o, n), :], preferred_element_type=F32)
    o_ref[...] = (x + s * (gg * jax.nn.sigmoid(gg))).astype(BF16)


@jax.jit
def pallas_recurrent_scan__compressed_kv_cla__dense_activation_gelu__decode_kernel(
    A_x: jax.Array,
    A_c_kv: jax.Array,
    A_w_q: jax.Array,
    A_w_uk: jax.Array,
    A_w_uv: jax.Array,
    A_w_o: jax.Array,
    B_x: jax.Array,
    B_w1: jax.Array,
    B_b1: jax.Array,
    B_w2: jax.Array,
    B_b2: jax.Array,
):
    del B_x
    out = pl.pallas_call(
        _kernel,
        out_shape=jax.ShapeDtypeStruct((B, M), BF16),
        in_specs=[pl.BlockSpec(memory_space=pltpu.HBM)] * 10,
        out_specs=pl.BlockSpec(memory_space=pltpu.VMEM),
        scratch_shapes=[
            pltpu.VMEM((B, M), BF16), pltpu.VMEM((F,), BF16), pltpu.VMEM((M,), BF16),
            pltpu.VMEM((B, SK, DC), BF16),
            pltpu.VMEM((M, H, D), BF16), pltpu.VMEM((DC, H, D), BF16), pltpu.VMEM((DC, H, D), BF16),
            pltpu.VMEM((H, D, M), BF16), pltpu.VMEM((M, F), BF16), pltpu.VMEM((F, M), BF16),
            pltpu.VMEM((B, M), F32), pltpu.SMEM((B, M), F32),
            pltpu.VMEM((DC * 8 + 8, 128), F32),
            pltpu.VMEM((B * H, DC), BF16), pltpu.VMEM((B * H, DC), F32),
            pltpu.VMEM((B * H, 128), F32), pltpu.VMEM((B * H, 128), F32),
            pltpu.VMEM((B * H, 128 * H), BF16),
            pltpu.SemaphoreType.DMA((AHEAD,)), pltpu.SemaphoreType.DMA((2,)),
        ],
        compiler_params=pltpu.CompilerParams(vmem_limit_bytes=100 * 1024 * 1024),
    )(A_x.reshape(B, M), A_c_kv, A_w_q, A_w_uk, A_w_uv, A_w_o, B_w1, B_b1, B_w2, B_b2)
    return out.reshape(B, 1, M)
```
